```python
import os as _os
_os.environ.setdefault("JAX_PLATFORMS", "cpu")
import jax
import jax.numpy as jnp

def _softmax(x, axis=-1):
    return jax.nn.softmax(x, axis=axis)
def _gelu(x):
    return jax.nn.gelu(x, approximate=True)
def _silu(x):
    return jax.nn.silu(x)
def _sigmoid(x):
    return jax.nn.sigmoid(x)
def _layernorm(x, axis=-1, eps=1e-5):
    m = jnp.mean(x, axis=axis, keepdims=True)
    v = jnp.var(x, axis=axis, keepdims=True)
    return (x - m) / jnp.sqrt(v + eps)
def _scatter_add(tgt, idx, src, axis=0):
    return tgt.at[idx].add(src)
def _segment_sum(src, seg, n):
    return jax.ops.segment_sum(src, seg, n)
class _Rng:
    def __init__(self, key):
        self._k = key
    def _next(self):
        self._k, sub = jax.random.split(self._k)
        return sub
    def normal(self, shape):
        return jax.random.normal(self._next(), shape, dtype=jnp.bfloat16)
    def randint(self, lo, hi, shape):
        return jax.random.randint(self._next(), shape, lo, hi, dtype=jnp.int32)
    def uniform(self, shape, lo=0.0, hi=1.0):
        return jax.random.uniform(self._next(), shape, jnp.bfloat16, lo, hi)
    def permutation(self, n):
        return jax.random.permutation(self._next(), n)


kernel_name = 'concat_heads__linear_attn_block__sliding_local_dilated__prompt'

def setup_inputs():
    _rng = _Rng(jax.random.key(int.from_bytes(__import__("os").urandom(4), "little")))
    _w = (lambda a: (lambda t: t.astype(jnp.bfloat16) if jnp.issubdtype(t.dtype, jnp.floating) else t)(jnp.asarray(a)))
    def _A_setup():
        B, S, D = 1, 2048, 576
        return {
            "x": _w((lambda *s: _rng.normal(s) * 0.05)(B, S, D)),
            "wqkv": _w((lambda *s: _rng.normal(s) * 1.6)(D, 3 * D)),
            "wo": _w((lambda *s: _rng.normal(s) * 0.4)(D, D)),
        }
    _A_in = _A_setup()

    def _B_setup():
        B, S, D = 1, 2048, 576
        return {
            "x": _w((lambda *s: _rng.normal(s) * 0.2)(B, S, D)),
            "wqkv": _w((lambda *s: _rng.normal(s) * 0.2)(D, 3 * D)),
            "wo": _w((lambda *s: _rng.normal(s) * 0.05)(D, D)),
        }
    _B_in = _B_setup()

    return {
        "A_x": _A_in["x"],
        "A_wqkv": _A_in["wqkv"],
        "A_wo": _A_in["wo"],
        "B_x": _B_in["x"],
        "B_wqkv": _B_in["wqkv"],
        "B_wo": _B_in["wo"],
    }

def reference(A_x, A_wqkv, A_wo, B_x, B_wqkv, B_wo):
    def _A_ref(x, wqkv, wo):
        B, S, D = x.shape
        H = 32; Dh = D // H
        qkv = (lambda x, *d: x.transpose(*d))((x @ wqkv).reshape(B, S, 3, H, Dh), 2, 0, 3, 1, 4)
        q, k, v = qkv[0], qkv[1], qkv[2]
        phi = lambda t: jnp.where(t > 0, t + 1, jnp.exp(t)) + 1e-6
        pq, pk = phi(q), phi(k)
        kv = jnp.einsum("bhsd,bhse->bhde", pk, v)
        z = jnp.einsum("bhsd->bhd", pk)
        num = jnp.einsum("bhqd,bhde->bhqe", pq, kv)
        den = jnp.einsum("bhqd,bhd->bhq", pq, z)[..., None] + 1e-6
        o = num / den
        return (lambda x, *d: x.transpose(*d))(o, 0, 2, 1, 3).reshape(B, S, D) @ wo

    def _B_ref(x, wqkv, wo):
        B, S, D = x.shape
        H = 32; Dh = D // H
        W, dil = 8, 2
        qkv = (lambda x, *d: x.transpose(*d))((x @ wqkv).reshape(B, S, 3, H, Dh), 2, 0, 3, 1, 4)
        q, k, v = qkv[0], qkv[1], qkv[2]
        scale = Dh ** -0.5
        pos = jnp.arange(S)
        off = jnp.arange(W) * dil
        idx = pos[:, None] - off[None, :]
        mask = idx >= 0
        idx_c = jnp.where(mask, idx, 0).reshape(-1)
        kg = k[:, :, idx_c, :].reshape(B, H, S, W, Dh)
        vg = v[:, :, idx_c, :].reshape(B, H, S, W, Dh)
        logits = jnp.einsum("bhsd,bhswd->bhsw", q, kg) * scale
        logits = jnp.where(mask[None, None, :, :], logits, -1e9)
        attn = _softmax(logits, axis=-1)
        o = jnp.einsum("bhsw,bhswd->bhsd", attn, vg)
        return (lambda x, *d: x.transpose(*d))(o, 0, 2, 1, 3).reshape(B, S, D) @ wo

    a = _A_ref(A_x, A_wqkv, A_wo)
    b = _B_ref(B_x, B_wqkv, B_wo)
    return jnp.concatenate([a, b], axis=-1)
```

```python
import functools

import jax
import jax.numpy as jnp
import numpy as np
from jax import lax
from jax.experimental import pallas as pl
from jax.experimental.pallas import tpu as pltpu

S = 2048
D = 576
H = 32
DH = 18
W = 8
DIL = 2
SB = 512
NB = S // SB
T = SB // 128
F32 = jnp.float32
BF16 = jnp.bfloat16
LOG2E = 1.4426950408889634

NT_DIMS = (((1,), (1,)), ((), ()))
TN_DIMS = (((0,), (0,)), ((), ()))


def _starts(order, blk):
    if order == "nat16":
        g, dh = divmod(blk, DH)
        s0 = 288 * g + dh
        return (s0, s0 + 8 * DH, DH)
    if order == "eo16":
        g, dh = divmod(blk, DH)
        s0 = 288 * g + dh
        return (s0, s0 + DH, 2 * DH)
    if order == "g8":
        g, m = divmod(blk, DH // 2)
        s0 = 144 * g + 2 * m
        return (s0, s0 + 1, DH)
    raise ValueError(order)


def _stage_transposed(w_ref, stage, tiles):
    for t in tiles:
        c0 = 128 * t
        nc = min(128, 3 * D - c0)
        wt = w_ref[:, c0:c0 + nc].astype(F32).T
        for u in range(4):
            stage[u, c0:c0 + nc, :] = wt[:, 128 * u:128 * u + 128]
        stage[4, c0:c0 + nc, 0:64] = wt[:, 512:576]


def _gather_rows(stage, base, order, dst):
    for blk in range(36):
        s0, s1, st = _starts(order, blk)
        for u in range(5):
            a = stage[u, pl.ds(base + s0, 8, stride=st), :]
            b = stage[u, pl.ds(base + s1, 8, stride=st), :]
            v = jnp.concatenate([a, b], axis=0).astype(BF16)
            if u < 4:
                dst[16 * blk:16 * blk + 16, 128 * u:128 * u + 128] = v
            else:
                dst[16 * blk:16 * blk + 16, 512:576] = v[:, 0:64]


def _phi(t):
    return jnp.where(t > 0, t + 1.0, jnp.exp(t)) + 1e-6


def _kernel(xa_hbm, wa_hbm, woa_hbm, xb_hbm, wb_hbm, wob_hbm, out_hbm,
            xa, xb, wa, wb, woa, wob,
            stage_a, stage_b, stage_o,
            wk_a, wq_a, wq_b, wk_b, wv_b, wo_b, m_a,
            g_acc, z_acc, zb,
            q_s, kp_s, vp_s, p_s, o_s, a_s, outbuf,
            sem_in, sem_out):
    def cp(src, dst, i):
        return pltpu.make_async_copy(src, dst, sem_in.at[i])

    c_wa = cp(wa_hbm, wa, 0)
    c_wb = cp(wb_hbm, wb, 1)
    c_woa = cp(woa_hbm, woa, 2)
    c_wob = cp(wob_hbm, wob, 3)
    c_xa = [cp(xa_hbm.at[:, pl.ds(i * SB, SB)], xa.at[i], 4 + i) for i in range(NB)]
    c_xb = [cp(xb_hbm.at[:, pl.ds(i * SB, SB)], xb.at[i], 4 + NB + i) for i in range(NB)]

    c_wa.start()
    for c in c_xa:
        c.start()
    c_wb.start()
    c_woa.start()
    c_wob.start()
    for c in c_xb:
        c.start()

    c_wa.wait()
    _stage_transposed(wa, stage_a, range(0, 9))
    _gather_rows(stage_a, D, "g8", wk_a)
    _gather_rows(stage_a, 0, "g8", wq_a)

    for i in range(NB):
        c_xa[i].wait()
        x = xa[i]
        kt = jnp.dot(wk_a[...], x, preferred_element_type=F32)
        pk = _phi(kt)
        zsum = pk[:, 0:128]
        for j in range(1, T):
            zsum = zsum + pk[:, 128 * j:128 * j + 128]
        gblk = lax.dot_general(pk.astype(BF16), x, NT_DIMS, preferred_element_type=F32)
        if i == 0:
            z_acc[...] = zsum
            g_acc[...] = gblk
        else:
            z_acc[...] += zsum
            g_acc[...] += gblk

    c_wb.wait()
    _stage_transposed(wb, stage_b, range(0, 14))
    _gather_rows(stage_b, 0, "eo16", wq_b)
    _gather_rows(stage_b, D, "nat16", wk_b)
    _gather_rows(stage_b, 2 * D, "nat16", wv_b)
    c_wob.wait()
    wo32 = wob[...].astype(F32)
    for u in range(4):
        stage_o[u] = wo32[:, 128 * u:128 * u + 128]
    stage_o[4, :, 0:64] = wo32[:, 512:576]
    _gather_rows(stage_o, 0, "eo16", wo_b)

    c_woa.wait()
    zcol = jnp.sum(z_acc[...], axis=1, keepdims=True)
    zb[...] = jnp.broadcast_to(zcol, (D, 128))
    for g in range(4):
        c0 = 128 * g
        nc = min(256, D - c0)
        gb = g_acc[144 * g:144 * g + 144, :].astype(BF16)
        kv = jnp.dot(gb, wa[:, 2 * D + c0:2 * D + c0 + nc], preferred_element_type=F32)
        row = lax.broadcasted_iota(jnp.int32, (144, nc), 0)
        col = lax.broadcasted_iota(jnp.int32, (144, nc), 1) + c0
        rel = col - DH * (8 * g + (row & 7))
        kv = jnp.where((rel >= 0) & (rel < DH), kv, 0.0)
        mg = jnp.dot(kv.astype(BF16), woa[c0:c0 + nc, :], preferred_element_type=F32)
        m_a[144 * g:144 * g + 144, :] = mg.astype(BF16)

    zero_tile = jnp.zeros((D // 2, 128), jnp.int32)
    kp_s[0] = zero_tile
    vp_s[0] = zero_tile

    lane = lax.broadcasted_iota(jnp.int32, (1, 8, 128), 2)
    lane2 = lax.broadcasted_iota(jnp.int32, (8, 128), 1)
    himask = jnp.int32(-65536)

    def shifted(ext, w):
        if w == 0:
            return ext[1:]
        r = pltpu.roll(ext, DIL * w, 2)
        return jnp.where(lane < DIL * w, r[:-1], r[1:])

    def unpack(wd):
        lo = pltpu.bitcast(wd << 16, F32)
        hi = pltpu.bitcast(wd & himask, F32)
        return lo, hi

    def block(i, carry):
        pltpu.make_async_copy(xb_hbm.at[:, pl.ds(0, SB)], xb.at[i], sem_in.at[4 + NB + i]).wait()
        x = xb[i]
        t0 = i * T
        qt = jnp.dot(wq_b[...], x, preferred_element_type=F32)
        for j in range(T):
            q_s[j] = qt[:, 128 * j:128 * j + 128]
        kt = jnp.dot(wk_b[...], x, preferred_element_type=F32)
        kpk = pltpu.bitcast(kt.astype(BF16), jnp.int32)
        for j in range(T):
            kp_s[t0 + 1 + j] = kpk[:, 128 * j:128 * j + 128]
        vt = jnp.dot(wv_b[...], x, preferred_element_type=F32)
        vpk = pltpu.bitcast(vt.astype(BF16), jnp.int32)
        for j in range(T):
            vp_s[t0 + 1 + j] = vpk[:, 128 * j:128 * j + 128]

        qa = _phi(jnp.dot(wq_a[...], xa[i], preferred_element_type=F32))
        for g in range(4):
            den = None
            for dh in range(DH):
                r0 = 144 * g + 8 * dh
                zr = zb[r0:r0 + 8, :]
                zr = jnp.concatenate([zr] * T, axis=1)
                pr = qa[r0:r0 + 8, :] * zr
                den = pr if den is None else den + pr
            inv = 1.0 / (den + 1e-6)
            for m in range(DH // 2):
                r0 = 144 * g + 16 * m
                a2 = qa[r0:r0 + 16, :] * jnp.concatenate([inv, inv], axis=0)
                a_s[r0:r0 + 16, :] = a2.astype(BF16)

        scale = (DH ** -0.5) * LOG2E
        for G in range(2):
            logits = []
            for w in range(W):
                acc_lo = acc_hi = None
                for dh in range(DH):
                    wr = 144 * G + 8 * dh
                    ext = kp_s[pl.ds(t0, T + 1), wr:wr + 8, :]
                    klo, khi = unpack(shifted(ext, w))
                    qr = 288 * G + 16 * dh
                    plo = q_s[:, qr:qr + 8, :] * klo
                    phi_ = q_s[:, qr + 8:qr + 16, :] * khi
                    acc_lo = plo if acc_lo is None else acc_lo + plo
                    acc_hi = phi_ if acc_hi is None else acc_hi + phi_
                logits.append((acc_lo, acc_hi))
            for half in range(2):
                ls = []
                for w in range(W):
                    l = logits[w][half] * scale
                    if w > 0:
                        first = jnp.where(lane2 + i * SB < DIL * w, -1e9, l[0])
                        l = jnp.concatenate([first[None], l[1:]], axis=0) if T > 1 else first[None]
                    ls.append(l)
                m = ls[0]
                for w in range(1, W):
                    m = jnp.maximum(m, ls[w])
                es = [jnp.exp2(l - m) for l in ls]
                ssum = es[0]
                for w in range(1, W):
                    ssum = ssum + es[w]
                inv = 1.0 / ssum
                for w in range(W):
                    p_s[G, w, half] = es[w] * inv
        for G in range(2):
            for dh in range(DH):
                wr = 144 * G + 8 * dh
                ext = vp_s[pl.ds(t0, T + 1), wr:wr + 8, :]
                acc_lo = acc_hi = None
                for w in range(W):
                    vlo, vhi = unpack(shifted(ext, w))
                    plo = p_s[G, w, 0] * vlo
                    phi_ = p_s[G, w, 1] * vhi
                    acc_lo = plo if acc_lo is None else acc_lo + plo
                    acc_hi = phi_ if acc_hi is None else acc_hi + phi_
                r0 = 288 * G + 16 * dh
                o_s[:, r0:r0 + 16, :] = jnp.concatenate([acc_lo, acc_hi], axis=1).astype(BF16)

        oa = lax.dot_general(m_a[...], a_s[...], TN_DIMS, preferred_element_type=F32)
        ob_in = jnp.concatenate([o_s[j] for j in range(T)], axis=1)
        ob = lax.dot_general(wo_b[...], ob_in, TN_DIMS, preferred_element_type=F32)
        ot = jnp.concatenate([oa.astype(BF16), ob.astype(BF16)], axis=0)
        outbuf[i] = ot.T
        pltpu.make_async_copy(outbuf.at[i], out_hbm.at[pl.ds(i * SB, SB), :], sem_out.at[i]).start()
        return carry

    lax.fori_loop(0, NB, block, 0)
    for i in range(NB):
        pltpu.make_async_copy(outbuf.at[i], out_hbm.at[pl.ds(i * SB, SB), :], sem_out.at[i]).wait()


@jax.jit
def pallas_concat_heads__linear_attn_block__sliding_local_dilated__prompt_kernel(
    A_x: jax.Array,
    A_wqkv: jax.Array,
    A_wo: jax.Array,
    B_x: jax.Array,
    B_wqkv: jax.Array,
    B_wo: jax.Array,
):
    xa_t = jnp.swapaxes(A_x, 1, 2).reshape(D, S)
    xb_t = jnp.swapaxes(B_x, 1, 2).reshape(D, S)
    any_spec = pl.BlockSpec(memory_space=pl.ANY)
    vm = pltpu.VMEM
    scratch = [
        vm((NB, D, SB), BF16), vm((NB, D, SB), BF16),
        vm((D, 3 * D), BF16), vm((D, 3 * D), BF16), vm((D, D), BF16), vm((D, D), BF16),
        vm((5, 9 * 128, 128), F32), vm((5, 3 * D, 128), F32), vm((5, D, 128), F32),
        vm((D, D), BF16), vm((D, D), BF16), vm((D, D), BF16), vm((D, D), BF16), vm((D, D), BF16),
        vm((D, D), BF16), vm((D, D), BF16),
        vm((D, D), F32), vm((D, 128), F32), vm((D, 128), F32),
        vm((T, D, 128), F32), vm((1 + S // 128, D // 2, 128), jnp.int32), vm((1 + S // 128, D // 2, 128), jnp.int32),
        vm((2, W, 2, T, 8, 128), F32), vm((T, D, 128), BF16), vm((D, SB), BF16),
        vm((NB, SB, 2 * D), BF16),
        pltpu.SemaphoreType.DMA((4 + 2 * NB,)), pltpu.SemaphoreType.DMA((NB,)),
    ]
    out = pl.pallas_call(
        _kernel,
        out_shape=jax.ShapeDtypeStruct((S, 2 * D), BF16),
        in_specs=[any_spec] * 6,
        out_specs=any_spec,
        scratch_shapes=scratch,
        compiler_params=pltpu.CompilerParams(vmem_limit_bytes=110 * 1024 * 1024),
    )(xa_t, A_wqkv, A_wo, xb_t, B_wqkv, B_wo)
    return out.reshape(1, S, 2 * D)
```

```python
import jax
import jax.numpy as jnp
from jax import lax
from jax.experimental import pallas as pl
from jax.experimental.pallas import tpu as pltpu

S = 2048
D = 576
DH = 18
W = 8
DIL = 2
SB = 512
NB = S // SB
T = SB // 128
TS = 2
GR = 8 * DH
X0 = 256
QSTEP = 120
F32 = jnp.float32
BF16 = jnp.bfloat16
I32 = jnp.int32
LOG2E = 1.4426950408889634
NT_DIMS = (((1,), (1,)), ((), ()))


def _phi(t):
    return jnp.where(t > 0, t + 1.0, jnp.exp(t)) + 1e-6


def _pack(lo, hi):
    return pltpu.bitcast(pltpu.pack_elementwise([lo, hi], packed_dtype=BF16), I32)


def _unpack(wd):
    return pltpu.bitcast(wd << 16, F32), pltpu.bitcast(wd & jnp.int32(-65536), F32)


def _head(idx):
    return jnp.floor((idx.astype(F32) + 0.5) * (1.0 / DH))


def _transpose_tiles(w_ref, dst, tiles):
    for t in tiles:
        c0 = 128 * t
        nc = min(128, w_ref.shape[1] - c0)
        dst[c0:c0 + nc, :] = w_ref[:, c0:c0 + nc].T


def _kernel(xa_hbm, wa_hbm, woa_hbm, xb_hbm, wb_hbm, wob_hbm, out_hbm,
            xa, xb, wa, wb, woa, wob, wt_a, wt_b, wot_b, mt_a,
            g_acc, gr_acc, z_acc, zb, zp,
            q_s, kp_s, vp_s, o_s, a_s, outbuf, sem_in, sem_out):
    def cols(src, dst, c0, nc, k):
        return pltpu.make_async_copy(src.at[:, pl.ds(c0, nc)], dst.at[:, pl.ds(c0, nc)], sem_in.at[k])

    def xblk(src, dst, i, k):
        return pltpu.make_async_copy(src.at[:, pl.ds(i * SB, SB)], dst.at[i], sem_in.at[k])

    c_wk = [cols(wa_hbm, wa, 128 * t, 128, t - 4) for t in range(4, 9)]
    c_x0 = [cols(xa_hbm, xa.at[0], 0, X0, 5), cols(xa_hbm, xa.at[0], X0, SB - X0, 6)]
    c_waq = cols(wa_hbm, wa, 0, 512, 7)
    c_wav = cols(wa_hbm, wa, 2 * D, D, 8)
    c_wb = pltpu.make_async_copy(wb_hbm, wb, sem_in.at[9])
    c_woa = pltpu.make_async_copy(woa_hbm, woa, sem_in.at[10])
    c_wob = pltpu.make_async_copy(wob_hbm, wob, sem_in.at[11])
    c_xa = [xblk(xa_hbm, xa, i, 11 + i) for i in range(1, NB)]
    c_xb = [xblk(xb_hbm, xb, i, 11 + NB + i) for i in range(NB)]

    for c in c_wk + c_x0:
        c.start()
    for t in range(4, 9):
        c_wk[t - 4].wait()
        _transpose_tiles(wa, wt_a, [t])
        if t == 6:
            for c in [c_xa[0], c_waq, c_xa[1], c_xa[2], c_wb, c_wob, c_wav, c_woa] + c_xb:
                c.start()

    def a1(i, c0=0, nc=SB):
        kt = jnp.dot(wt_a[D:2 * D, :], xa[i, :, c0:c0 + nc], preferred_element_type=F32)
        pk = _phi(kt)
        zsum = pk[:, 0:128]
        for j in range(1, nc // 128):
            zsum = zsum + pk[:, 128 * j:128 * j + 128]
        pkb = pk.astype(BF16)
        gblk = lax.dot_general(pkb, xa[i, 0:512, c0:c0 + nc], NT_DIMS, preferred_element_type=F32)
        grem = lax.dot_general(xa[i, 512:D, c0:c0 + nc], pkb, NT_DIMS, preferred_element_type=F32)
        if i == 0 and c0 == 0:
            z_acc[...] = zsum
            g_acc[...] = gblk
            gr_acc[...] = grem
        else:
            z_acc[...] += zsum
            g_acc[...] += gblk
            gr_acc[...] += grem

    c_x0[0].wait()
    a1(0, 0, X0)
    c_x0[1].wait()
    c_xa[0].wait()
    a1(0, X0, SB - X0)
    a1(1)
    for c in [c_waq, c_xa[1], c_xa[2], c_wb, c_wob]:
        c.wait()
    _transpose_tiles(wa, wt_a, range(0, 4))
    _transpose_tiles(wb, wt_b, range(0, 7))
    a1(2)
    _transpose_tiles(wb, wt_b, range(7, 14))
    _transpose_tiles(wob, wot_b, range(0, 5))
    a1(3)
    for c in [c_wav, c_woa] + c_xb:
        c.wait()

    zb[...] = jnp.broadcast_to(jnp.sum(z_acc[...], axis=1, keepdims=True), (D, 128))
    for g in range(4):
        for dh in range(DH):
            r0 = GR * g + 8 * dh
            zp[r0:r0 + 8, :] = zb[pl.ds(GR * g + dh, 8, stride=DH), :]
    grt = gr_acc[...].T
    bands = [(0, 144), (112, 272), (240, 400), (368, 528), (496, 576)]
    kvs = []
    for t, (lo, hi) in enumerate(bands):
        c0 = 128 * t
        nc = min(128, D - c0)
        gb = jnp.concatenate([g_acc[lo:hi, :], grt[lo:hi, :]], axis=1).astype(BF16)
        kv = jnp.dot(gb, wa[:, 2 * D + c0:2 * D + c0 + nc], preferred_element_type=F32)
        row = lax.broadcasted_iota(I32, (hi - lo, nc), 0) + lo
        col = lax.broadcasted_iota(I32, (hi - lo, nc), 1) + c0
        kvs.append(jnp.where(_head(row) == _head(col), kv, 0.0).astype(BF16))
    edges = [0, 112, 144, 240, 272, 368, 400, 496, 528, 576]
    msegs = []
    for r0, r1 in zip(edges[:-1], edges[1:]):
        ts = [t for t, (lo, hi) in enumerate(bands) if lo <= r0 and r1 <= hi]
        lhs = jnp.concatenate([kvs[t][r0 - bands[t][0]:r1 - bands[t][0], :] for t in ts], axis=1)
        rhs = woa[128 * ts[0]:min(D, 128 * ts[-1] + 128), :]
        msegs.append(jnp.dot(lhs, rhs, preferred_element_type=F32).astype(BF16))
    mt_a[...] = jnp.concatenate(msegs, axis=0).T

    zero_tile = jnp.zeros((D // 2, 128), I32)
    kp_s[0] = zero_tile
    vp_s[0] = zero_tile
    lane3 = lax.broadcasted_iota(I32, (1, 8, 128), 2)
    lane2 = lax.broadcasted_iota(I32, (8, 128), 1)
    scale = (DH ** -0.5) * LOG2E

    def shifted(ext, w):
        if w == 0:
            return ext[1:]
        r = pltpu.roll(ext, DIL * w, 2)
        return jnp.where(lane3 < DIL * w, r[:-1], r[1:])

    def out_copy(i):
        return pltpu.make_async_copy(outbuf.at[i], out_hbm.at[pl.ds(i * SB, SB), :], sem_out.at[i])

    def qrows(r0, tiles=slice(None)):
        return pltpu.bitcast(q_s[tiles, pl.ds(r0, 8, stride=DH), :], F32)

    def block(i, last):
        t0 = i * T
        prev = (i + NB - 1) % NB

        for c in range(9):
            wds = jnp.concatenate([q_s[j, 64 * c:64 * c + 64, :] for j in range(T)], axis=1)
            outbuf[prev, :, 128 * c:128 * c + 128] = pltpu.bitcast(wds, BF16).T

        qa = _phi(jnp.dot(wt_a[0:D, :], xa[i], preferred_element_type=F32))
        for j in range(T):
            q_s[j] = pltpu.bitcast(qa[:, 128 * j:128 * j + 128], I32)
        for g in range(4):
            den = None
            for dh in range(DH):
                r0 = GR * g + 8 * dh
                pr = qrows(GR * g + dh) * zp[r0:r0 + 8, :][None]
                den = pr if den is None else den + pr
            inv = 1.0 / (den + 1e-6)
            for m in range(DH // 2):
                lo = qrows(GR * g + 2 * m) * inv
                hi = qrows(GR * g + 2 * m + 1) * inv
                a_s[:, pl.ds(GR // 2 * g + m, 8, stride=DH // 2), :] = _pack(lo, hi)

        x = xb[i]
        for g in range(4):
            r, rw, rq = GR * g, GR // 2 * g, QSTEP * g
            lhs = jnp.concatenate([wt_b[c * D + r:c * D + r + GR, :] for c in range(3)], axis=0)
            qkv = jnp.dot(lhs, x, preferred_element_type=F32)
            kvp = pltpu.bitcast(qkv[GR:3 * GR, :].astype(BF16), I32)
            for j in range(T):
                lanes = slice(128 * j, 128 * j + 128)
                q_s[j, rq:rq + GR, :] = pltpu.bitcast(qkv[0:GR, lanes], I32)
                kp_s[t0 + 1 + j, rw:rw + GR // 2, :] = kvp[0:GR // 2, lanes]
                vp_s[t0 + 1 + j, rw:rw + GR // 2, :] = kvp[GR // 2:GR, lanes]

            if last and g == 3:
                out_copy(prev).start()
                out_copy(0).wait()

            for sb in range(T // TS):
                tl = pl.ds(sb * TS, TS)
                te = pl.ds(t0 + sb * TS, TS + 1)
                acc = [None] * W
                for m in range(DH // 2):
                    ext = kp_s[te, pl.ds(rw + m, 8, stride=DH // 2), :]
                    qlo = qrows(rq + 2 * m, tl)
                    qhi = qrows(rq + 2 * m + 1, tl)
                    for w in range(W):
                        klo, khi = _unpack(shifted(ext, w))
                        pr = qlo * klo + qhi * khi
                        acc[w] = pr if acc[w] is None else acc[w] + pr
                ls = []
                for w in range(W):
                    l = acc[w] * scale
                    if w > 0 and sb == 0:
                        l0 = jnp.where(lane2 + i * SB < DIL * w, -1e9 * LOG2E, l[0])
                        l = jnp.concatenate([l0[None], l[1:]], axis=0)
                    ls.append(l)
                mx = ls[0]
                for w in range(1, W):
                    mx = jnp.maximum(mx, ls[w])
                es = [jnp.exp2(l - mx) for l in ls]
                ssum = es[0]
                for w in range(1, W):
                    ssum = ssum + es[w]
                inv = 1.0 / ssum
                ps = [e * inv for e in es]
                for m in range(DH // 2):
                    ext = vp_s[te, pl.ds(rw + m, 8, stride=DH // 2), :]
                    olo = ohi = None
                    for w in range(W):
                        vlo, vhi = _unpack(shifted(ext, w))
                        olo = ps[w] * vlo if olo is None else olo + ps[w] * vlo
                        ohi = ps[w] * vhi if ohi is None else ohi + ps[w] * vhi
                    o_s[tl, pl.ds(rw + m, 8, stride=DH // 2), :] = _pack(olo, ohi)

        a_in = jnp.concatenate([pltpu.bitcast(a_s[j], BF16) for j in range(T)], axis=1)
        b_in = jnp.concatenate([pltpu.bitcast(o_s[j], BF16) for j in range(T)], axis=1)
        oa = jnp.dot(mt_a[...], a_in, preferred_element_type=F32).astype(BF16)

        def b_out(r0, r1):
            return jnp.dot(wot_b[r0:r1, :], b_in, preferred_element_type=F32).astype(BF16)

        if not last:
            ot = pltpu.bitcast(jnp.concatenate([oa, b_out(0, D)], axis=0), I32)
            for j in range(T):
                q_s[j] = ot[:, 128 * j:128 * j + 128]

            @pl.when(i > 0)
            def _():
                out_copy(prev).start()
            return

        cps = [pltpu.make_async_copy(outbuf.at[i, :, pl.ds(c0, nc)],
                                     out_hbm.at[pl.ds(i * SB, SB), pl.ds(c0, nc)], sem_out.at[NB - 1 + k])
               for k, (c0, nc) in enumerate([(0, 512), (512, 256), (768, 256), (1024, 128)])]
        ob0 = b_out(0, 192)
        outbuf[i, :, 0:512] = oa[0:512, :].T
        cps[0].start()
        out_copy(1).wait()
        ob1 = b_out(192, 448)
        outbuf[i, :, 512:768] = jnp.concatenate([oa[512:D, :], ob0], axis=0).T
        cps[1].start()
        out_copy(2).wait()
        ob2 = b_out(448, D)
        outbuf[i, :, 768:1024] = ob1.T
        cps[2].start()
        cps[0].wait()
        outbuf[i, :, 1024:1152] = ob2.T
        cps[3].start()
        for c in cps[1:]:
            c.wait()

    q_s[...] = jnp.zeros((T, D, 128), I32)

    def loop_body(i, carry):
        block(i, False)
        return carry

    lax.fori_loop(0, NB - 1, loop_body, 0)
    block(NB - 1, True)


@jax.jit
def pallas_concat_heads__linear_attn_block__sliding_local_dilated__prompt_kernel(
    A_x: jax.Array,
    A_wqkv: jax.Array,
    A_wo: jax.Array,
    B_x: jax.Array,
    B_wqkv: jax.Array,
    B_wo: jax.Array,
):
    xa_t = jnp.swapaxes(A_x, 1, 2).reshape(D, S)
    xb_t = jnp.swapaxes(B_x, 1, 2).reshape(D, S)
    any_spec = pl.BlockSpec(memory_space=pl.ANY)
    vm = pltpu.VMEM
    scratch = [
        vm((NB, D, SB), BF16), vm((NB, D, SB), BF16),
        vm((D, 3 * D), BF16), vm((D, 3 * D), BF16), vm((D, D), BF16), vm((D, D), BF16),
        vm((2 * D, D), BF16), vm((3 * D, D), BF16), vm((D, D), BF16), vm((D, D), BF16),
        vm((D, 512), F32), vm((D - 512, D), F32), vm((D, 128), F32),
        vm((D, 128), F32), vm((D, 128), F32),
        vm((T, D, 128), I32),
        vm((1 + S // 128, D // 2, 128), I32), vm((1 + S // 128, D // 2, 128), I32),
        vm((T, D // 2, 128), I32), vm((T, D // 2, 128), I32),
        vm((NB, SB, 2 * D), BF16),
        pltpu.SemaphoreType.DMA((11 + 2 * NB,)), pltpu.SemaphoreType.DMA((NB + 3,)),
    ]
    out = pl.pallas_call(
        _kernel,
        out_shape=jax.ShapeDtypeStruct((S, 2 * D), BF16),
        in_specs=[any_spec] * 6,
        out_specs=any_spec,
        scratch_shapes=scratch,
        compiler_params=pltpu.CompilerParams(
            vmem_limit_bytes=100 * 1024 * 1024, disable_semaphore_checks=True),
    )(xa_t, A_wqkv, A_wo, xb_t, B_wqkv, B_wo)
    return out.reshape(1, S, 2 * D)
```

```python
import jax
import jax.numpy as jnp
from jax import lax
from jax.experimental import pallas as pl
from jax.experimental.pallas import tpu as pltpu

S = 2048
D = 576
DH = 18
W = 8
DIL = 2
SB = 512
NB = S // SB
T = SB // 128
TS = 2
GR = 8 * DH
X0 = 256
QSTEP = 120
F32 = jnp.float32
BF16 = jnp.bfloat16
I32 = jnp.int32
LOG2E = 1.4426950408889634
NT_DIMS = (((1,), (1,)), ((), ()))


def _phi(t):
    return jnp.where(t > 0, t + 1.0, jnp.exp(t)) + 1e-6


def _pack(lo, hi):
    return pltpu.bitcast(pltpu.pack_elementwise([lo, hi], packed_dtype=BF16), I32)


def _unpack(wd):
    return pltpu.bitcast(wd << 16, F32), pltpu.bitcast(wd & jnp.int32(-65536), F32)


def _head(idx):
    return jnp.floor((idx.astype(F32) + 0.5) * (1.0 / DH))


def _transpose_tiles(w_ref, dst, tiles):
    for t in tiles:
        c0 = 128 * t
        nc = min(128, w_ref.shape[1] - c0)
        dst[c0:c0 + nc, :] = w_ref[:, c0:c0 + nc].T


def _kernel(xa_hbm, wa_hbm, woa_hbm, xb_hbm, wb_hbm, wob_hbm, out_hbm,
            xa, xb, wa, wb, woa, wob, wt_a, wt_b, wot_b, mt_a,
            g_acc, gr_acc, z_acc, zb, zp,
            q_s, kp_s, vp_s, o_s, a_s, outbuf, sem_in, sem_out):
    def cols(src, dst, c0, nc, k):
        return pltpu.make_async_copy(src.at[:, pl.ds(c0, nc)], dst.at[:, pl.ds(c0, nc)], sem_in.at[k])

    def xblk(src, dst, i, k):
        return pltpu.make_async_copy(src.at[:, pl.ds(i * SB, SB)], dst.at[i], sem_in.at[k])

    c_wk = [cols(wa_hbm, wa, 128 * t, 128, t - 4) for t in range(4, 9)]
    c_x0 = [cols(xa_hbm, xa.at[0], 0, X0, 5), cols(xa_hbm, xa.at[0], X0, SB - X0, 6)]
    c_waq = cols(wa_hbm, wa, 0, 512, 7)
    c_wav = cols(wa_hbm, wa, 2 * D, D, 8)
    c_wb = pltpu.make_async_copy(wb_hbm, wb, sem_in.at[9])
    c_woa = pltpu.make_async_copy(woa_hbm, woa, sem_in.at[10])
    c_wob = pltpu.make_async_copy(wob_hbm, wob, sem_in.at[11])
    c_xa = [xblk(xa_hbm, xa, i, 11 + i) for i in range(1, NB)]
    c_xb = [xblk(xb_hbm, xb, i, 11 + NB + i) for i in range(NB)]

    for c in c_wk + c_x0:
        c.start()
    for t in range(4, 9):
        c_wk[t - 4].wait()
        _transpose_tiles(wa, wt_a, [t])
        if t == 6:
            for c in [c_xa[0], c_waq, c_xa[1], c_xa[2], c_wb, c_wob, c_wav, c_woa] + c_xb:
                c.start()

    def a1(i, c0=0, nc=SB):
        kt = jnp.concatenate([jnp.dot(wt_a[D + r:D + r + 192, :], xa[i, :, c0:c0 + nc], preferred_element_type=F32)
                              for r in range(0, D, 192)], axis=0)
        pk = _phi(kt)
        zsum = pk[:, 0:128]
        for j in range(1, nc // 128):
            zsum = zsum + pk[:, 128 * j:128 * j + 128]
        pkb = pk.astype(BF16)
        gblk = jnp.concatenate([lax.dot_general(pkb[r:r + 192], xa[i, 0:512, c0:c0 + nc], NT_DIMS,
                                                preferred_element_type=F32) for r in range(0, D, 192)], axis=0)
        grem = lax.dot_general(xa[i, 512:D, c0:c0 + nc], pkb, NT_DIMS, preferred_element_type=F32)
        if i == 0 and c0 == 0:
            z_acc[...] = zsum
            g_acc[...] = gblk
            gr_acc[...] = grem
        else:
            z_acc[...] += zsum
            g_acc[...] += gblk
            gr_acc[...] += grem

    c_x0[0].wait()
    a1(0, 0, X0)
    c_x0[1].wait()
    c_xa[0].wait()
    a1(0, X0, SB - X0)
    a1(1)
    for c in [c_waq, c_xa[1], c_xa[2], c_wb, c_wob]:
        c.wait()
    _transpose_tiles(wa, wt_a, range(0, 4))
    _transpose_tiles(wb, wt_b, range(0, 7))
    a1(2)
    _transpose_tiles(wb, wt_b, range(7, 14))
    _transpose_tiles(wob, wot_b, range(0, 5))
    a1(3)
    for c in [c_wav, c_woa] + c_xb:
        c.wait()

    zb[...] = jnp.broadcast_to(jnp.sum(z_acc[...], axis=1, keepdims=True), (D, 128))
    for g in range(4):
        for dh in range(DH):
            r0 = GR * g + 8 * dh
            zp[r0:r0 + 8, :] = zb[pl.ds(GR * g + dh, 8, stride=DH), :]
    grt = gr_acc[...].T
    bands = [(0, 144), (112, 272), (240, 400), (368, 528), (496, 576)]
    kvs = []
    for t, (lo, hi) in enumerate(bands):
        c0 = 128 * t
        nc = min(128, D - c0)
        gb = jnp.concatenate([g_acc[lo:hi, :], grt[lo:hi, :]], axis=1).astype(BF16)
        kv = jnp.dot(gb, wa[:, 2 * D + c0:2 * D + c0 + nc], preferred_element_type=F32)
        row = lax.broadcasted_iota(I32, (hi - lo, nc), 0) + lo
        col = lax.broadcasted_iota(I32, (hi - lo, nc), 1) + c0
        kvs.append(jnp.where(_head(row) == _head(col), kv, 0.0).astype(BF16))
    edges = [0, 112, 144, 240, 272, 368, 400, 496, 528, 576]
    msegs = []
    for r0, r1 in zip(edges[:-1], edges[1:]):
        ts = [t for t, (lo, hi) in enumerate(bands) if lo <= r0 and r1 <= hi]
        lhs = jnp.concatenate([kvs[t][r0 - bands[t][0]:r1 - bands[t][0], :] for t in ts], axis=1)
        rhs = woa[128 * ts[0]:min(D, 128 * ts[-1] + 128), :]
        msegs.append(jnp.dot(lhs, rhs, preferred_element_type=F32).astype(BF16))
    mt_a[...] = jnp.concatenate(msegs, axis=0).T

    zero_tile = jnp.zeros((D // 2, 128), I32)
    kp_s[0] = zero_tile
    vp_s[0] = zero_tile
    lane3 = lax.broadcasted_iota(I32, (1, 8, 128), 2)
    lane2 = lax.broadcasted_iota(I32, (8, 128), 1)
    scale = (DH ** -0.5) * LOG2E

    def shifted(ext, w):
        if w == 0:
            return ext[1:]
        r = pltpu.roll(ext, DIL * w, 2)
        return jnp.where(lane3 < DIL * w, r[:-1], r[1:])

    def out_copy(i):
        return pltpu.make_async_copy(outbuf.at[i], out_hbm.at[pl.ds(i * SB, SB), :], sem_out.at[i])

    def qrows(r0, tiles=slice(None)):
        return pltpu.bitcast(q_s[tiles, pl.ds(r0, 8, stride=DH), :], F32)

    def block(i, last):
        t0 = i * T
        prev = (i + NB - 1) % NB

        for c in range(9):
            wds = jnp.concatenate([q_s[j, 64 * c:64 * c + 64, :] for j in range(T)], axis=1)
            outbuf[prev, :, 128 * c:128 * c + 128] = pltpu.bitcast(wds, BF16).T

        for r in range(0, D, D // 2):
            qa = _phi(jnp.dot(wt_a[r:r + D // 2, :], xa[i], preferred_element_type=F32))
            for j in range(T):
                q_s[j, r:r + D // 2, :] = pltpu.bitcast(qa[:, 128 * j:128 * j + 128], I32)
        for g in range(4):
            den = None
            for dh in range(DH):
                r0 = GR * g + 8 * dh
                pr = qrows(GR * g + dh) * zp[r0:r0 + 8, :][None]
                den = pr if den is None else den + pr
            inv = 1.0 / (den + 1e-6)
            for m in range(DH // 2):
                lo = qrows(GR * g + 2 * m) * inv
                hi = qrows(GR * g + 2 * m + 1) * inv
                a_s[:, pl.ds(GR // 2 * g + m, 8, stride=DH // 2), :] = _pack(lo, hi)

        x = xb[i]
        for g in range(4):
            r, rw, rq = GR * g, GR // 2 * g, QSTEP * g
            q, k, v = [jnp.dot(wt_b[c * D + r:c * D + r + GR, :], x, preferred_element_type=F32) for c in range(3)]
            kvp = pltpu.bitcast(jnp.concatenate([k, v], axis=0).astype(BF16), I32)
            for j in range(T):
                lanes = slice(128 * j, 128 * j + 128)
                q_s[j, rq:rq + GR, :] = pltpu.bitcast(q[:, lanes], I32)
                kp_s[t0 + 1 + j, rw:rw + GR // 2, :] = kvp[0:GR // 2, lanes]
                vp_s[t0 + 1 + j, rw:rw + GR // 2, :] = kvp[GR // 2:GR, lanes]

            if last and g == 3:
                out_copy(prev).start()
                out_copy(0).wait()

            for sb in range(T // TS):
                tl = pl.ds(sb * TS, TS)
                te = pl.ds(t0 + sb * TS, TS + 1)
                acc = [None] * W
                for m in range(DH // 2):
                    ext = kp_s[te, pl.ds(rw + m, 8, stride=DH // 2), :]
                    qlo = qrows(rq + 2 * m, tl)
                    qhi = qrows(rq + 2 * m + 1, tl)
                    for w in range(W):
                        klo, khi = _unpack(shifted(ext, w))
                        pr = qlo * klo + qhi * khi
                        acc[w] = pr if acc[w] is None else acc[w] + pr
                ls = []
                for w in range(W):
                    l = acc[w] * scale
                    if w > 0 and sb == 0:
                        l0 = jnp.where(lane2 + i * SB < DIL * w, -1e9 * LOG2E, l[0])
                        l = jnp.concatenate([l0[None], l[1:]], axis=0)
                    ls.append(l)
                mx = ls[0]
                for w in range(1, W):
                    mx = jnp.maximum(mx, ls[w])
                es = [jnp.exp2(l - mx) for l in ls]
                ssum = es[0]
                for w in range(1, W):
                    ssum = ssum + es[w]
                inv = 1.0 / ssum
                ps = [e * inv for e in es]
                for m in range(DH // 2):
                    ext = vp_s[te, pl.ds(rw + m, 8, stride=DH // 2), :]
                    olo = ohi = None
                    for w in range(W):
                        vlo, vhi = _unpack(shifted(ext, w))
                        olo = ps[w] * vlo if olo is None else olo + ps[w] * vlo
                        ohi = ps[w] * vhi if ohi is None else ohi + ps[w] * vhi
                    o_s[tl, pl.ds(rw + m, 8, stride=DH // 2), :] = _pack(olo, ohi)

        a_in = jnp.concatenate([pltpu.bitcast(a_s[j], BF16) for j in range(T)], axis=1)
        b_in = jnp.concatenate([pltpu.bitcast(o_s[j], BF16) for j in range(T)], axis=1)
        oa = jnp.dot(mt_a[...], a_in, preferred_element_type=F32).astype(BF16)

        def b_out(r0, r1):
            return jnp.dot(wot_b[r0:r1, :], b_in, preferred_element_type=F32).astype(BF16)

        if not last:
            ot = pltpu.bitcast(jnp.concatenate([oa, b_out(0, D)], axis=0), I32)
            for j in range(T):
                q_s[j] = ot[:, 128 * j:128 * j + 128]

            @pl.when(i > 0)
            def _():
                out_copy(prev).start()
            return

        cps = [pltpu.make_async_copy(outbuf.at[i, :, pl.ds(c0, nc)],
                                     out_hbm.at[pl.ds(i * SB, SB), pl.ds(c0, nc)], sem_out.at[NB - 1 + k])
               for k, (c0, nc) in enumerate([(0, 512), (512, 256), (768, 256), (1024, 128)])]
        ob0 = b_out(0, 192)
        outbuf[i, :, 0:512] = oa[0:512, :].T
        cps[0].start()
        out_copy(1).wait()
        ob1 = b_out(192, 448)
        outbuf[i, :, 512:768] = jnp.concatenate([oa[512:D, :], ob0], axis=0).T
        cps[1].start()
        out_copy(2).wait()
        ob2 = b_out(448, D)
        outbuf[i, :, 768:1024] = ob1.T
        cps[2].start()
        cps[0].wait()
        outbuf[i, :, 1024:1152] = ob2.T
        cps[3].start()
        for c in cps[1:]:
            c.wait()

    q_s[...] = jnp.zeros((T, D, 128), I32)

    def loop_body(i, carry):
        block(i, False)
        return carry

    lax.fori_loop(0, NB - 1, loop_body, 0)
    block(NB - 1, True)


@jax.jit
def pallas_concat_heads__linear_attn_block__sliding_local_dilated__prompt_kernel(
    A_x: jax.Array,
    A_wqkv: jax.Array,
    A_wo: jax.Array,
    B_x: jax.Array,
    B_wqkv: jax.Array,
    B_wo: jax.Array,
):
    xa_t = jnp.swapaxes(A_x, 1, 2).reshape(D, S)
    xb_t = jnp.swapaxes(B_x, 1, 2).reshape(D, S)
    any_spec = pl.BlockSpec(memory_space=pl.ANY)
    vm = pltpu.VMEM
    scratch = [
        vm((NB, D, SB), BF16), vm((NB, D, SB), BF16),
        vm((D, 3 * D), BF16), vm((D, 3 * D), BF16), vm((D, D), BF16), vm((D, D), BF16),
        vm((2 * D, D), BF16), vm((3 * D, D), BF16), vm((D, D), BF16), vm((D, D), BF16),
        vm((D, 512), F32), vm((D - 512, D), F32), vm((D, 128), F32),
        vm((D, 128), F32), vm((D, 128), F32),
        vm((T, D, 128), I32),
        vm((1 + S // 128, D // 2, 128), I32), vm((1 + S // 128, D // 2, 128), I32),
        vm((T, D // 2, 128), I32), vm((T, D // 2, 128), I32),
        vm((NB, SB, 2 * D), BF16),
        pltpu.SemaphoreType.DMA((11 + 2 * NB,)), pltpu.SemaphoreType.DMA((NB + 3,)),
    ]
    out = pl.pallas_call(
        _kernel,
        out_shape=jax.ShapeDtypeStruct((S, 2 * D), BF16),
        in_specs=[any_spec] * 6,
        out_specs=any_spec,
        scratch_shapes=scratch,
        compiler_params=pltpu.CompilerParams(
            vmem_limit_bytes=100 * 1024 * 1024, disable_semaphore_checks=True),
    )(xa_t, A_wqkv, A_wo, xb_t, B_wqkv, B_wo)
    return out.reshape(1, S, 2 * D)
```

```python
import jax
import jax.numpy as jnp
from jax import lax
from jax.experimental import pallas as pl
from jax.experimental.pallas import tpu as pltpu

S = 2048
D = 576
DH = 18
W = 8
DIL = 2
SB = 512
NB = S // SB
T = SB // 128
TS = 2
DP = D + 32
GR = 8 * DH
X0 = 256
QSTEP = 120
F32 = jnp.float32
BF16 = jnp.bfloat16
I32 = jnp.int32
LOG2E = 1.4426950408889634
NT_DIMS = (((1,), (1,)), ((), ()))


def _phi(t):
    return jnp.where(t > 0, t + 1.0, jnp.exp(t)) + 1e-6


def _unpack(wd):
    return pltpu.bitcast(wd << 16, F32), pltpu.bitcast(wd & jnp.int32(-65536), F32)


def _head(idx):
    return jnp.floor((idx.astype(F32) + 0.5) * (1.0 / DH))


def _transpose_tiles(w_ref, dst, tiles):
    for t in tiles:
        c0 = 128 * t
        nc = min(128, w_ref.shape[1] - c0)
        dst[c0:c0 + nc, :] = w_ref[:, c0:c0 + nc].T


def _kernel(xa_hbm, wa_hbm, woa_hbm, xb_hbm, wb_hbm, wob_hbm, out_hbm,
            xa, xb, wa, wb, woa, wob, wt_a, wt_b, wot_b, mt_a,
            g_acc, gr_acc, z_acc, zb, zp,
            q_s, kp_s, vp_s, o_s, a_s, outbuf, sem_in, sem_out):
    def cols(src, dst, c0, nc, k):
        return pltpu.make_async_copy(src.at[:, pl.ds(c0, nc)], dst.at[:, pl.ds(c0, nc)], sem_in.at[k])

    def xblk(src, dst, i, k):
        return pltpu.make_async_copy(src.at[:, pl.ds(i * SB, SB)], dst.at[i], sem_in.at[k])

    c_wk = [cols(wa_hbm, wa, 128 * t, 128, t - 4) for t in range(4, 9)]
    c_x0 = [cols(xa_hbm, xa.at[0], 0, X0, 5), cols(xa_hbm, xa.at[0], X0, SB - X0, 6)]
    c_waq = cols(wa_hbm, wa, 0, 512, 7)
    c_wav = cols(wa_hbm, wa, 2 * D, D, 8)
    c_wb = pltpu.make_async_copy(wb_hbm, wb, sem_in.at[9])
    c_woa = pltpu.make_async_copy(woa_hbm, woa, sem_in.at[10])
    c_wob = pltpu.make_async_copy(wob_hbm, wob, sem_in.at[11])
    c_xa = [xblk(xa_hbm, xa, i, 11 + i) for i in range(1, NB)]
    c_xb = [xblk(xb_hbm, xb, i, 11 + NB + i) for i in range(NB)]

    for c in c_wk + c_x0:
        c.start()
    for t in range(4, 9):
        c_wk[t - 4].wait()
        _transpose_tiles(wa, wt_a, [t])
        if t == 6:
            for c in [c_xa[0], c_waq, c_xa[1], c_xa[2], c_wb, c_wob, c_wav, c_woa] + c_xb:
                c.start()

    def a1(i, c0=0, nc=SB):
        kt = jnp.concatenate([jnp.dot(wt_a[D + r:D + r + 192, :], xa[i, :, c0:c0 + nc], preferred_element_type=F32)
                              for r in range(0, D, 192)], axis=0)
        pk = _phi(kt)
        zsum = pk[:, 0:128]
        for j in range(1, nc // 128):
            zsum = zsum + pk[:, 128 * j:128 * j + 128]
        pkb = pk.astype(BF16)
        gblk = jnp.concatenate([lax.dot_general(pkb[r:r + 192], xa[i, 0:512, c0:c0 + nc], NT_DIMS,
                                                preferred_element_type=F32) for r in range(0, D, 192)], axis=0)
        grem = lax.dot_general(xa[i, 512:D, c0:c0 + nc], pkb, NT_DIMS, preferred_element_type=F32)
        if i == 0 and c0 == 0:
            z_acc[...] = zsum
            g_acc[...] = gblk
            gr_acc[...] = grem
        else:
            z_acc[...] += zsum
            g_acc[...] += gblk
            gr_acc[...] += grem

    c_x0[0].wait()
    a1(0, 0, X0)
    c_x0[1].wait()
    c_xa[0].wait()
    a1(0, X0, SB - X0)
    a1(1)
    for c in [c_waq, c_xa[1], c_xa[2], c_wb, c_wob]:
        c.wait()
    _transpose_tiles(wa, wt_a, range(0, 4))
    _transpose_tiles(wb, wt_b, range(0, 7))
    a1(2)
    _transpose_tiles(wb, wt_b, range(7, 14))
    _transpose_tiles(wob, wot_b, range(0, 5))
    a1(3)
    for c in [c_wav, c_woa] + c_xb:
        c.wait()

    zb[0:D, :] = jnp.broadcast_to(jnp.sum(z_acc[...], axis=1, keepdims=True), (D, 128))
    for g in range(4):
        for dh in range(DH):
            r0 = GR * g + 8 * dh
            zp[r0:r0 + 8, :] = zb[pl.ds(GR * g + dh, 8, stride=DH), :]
    grt = gr_acc[...].T
    bands = [(0, 144), (112, 272), (240, 400), (368, 528), (496, 576)]
    kvs = []
    for t, (lo, hi) in enumerate(bands):
        c0 = 128 * t
        nc = min(128, D - c0)
        gb = jnp.concatenate([g_acc[lo:hi, :], grt[lo:hi, :]], axis=1).astype(BF16)
        kv = jnp.dot(gb, wa[:, 2 * D + c0:2 * D + c0 + nc], preferred_element_type=F32)
        row = lax.broadcasted_iota(I32, (hi - lo, nc), 0) + lo
        col = lax.broadcasted_iota(I32, (hi - lo, nc), 1) + c0
        kvs.append(jnp.where(_head(row) == _head(col), kv, 0.0).astype(BF16))
    edges = [0, 112, 144, 240, 272, 368, 400, 496, 528, 576]
    msegs = []
    for r0, r1 in zip(edges[:-1], edges[1:]):
        ts = [t for t, (lo, hi) in enumerate(bands) if lo <= r0 and r1 <= hi]
        lhs = jnp.concatenate([kvs[t][r0 - bands[t][0]:r1 - bands[t][0], :] for t in ts], axis=1)
        rhs = woa[128 * ts[0]:min(D, 128 * ts[-1] + 128), :]
        msegs.append(jnp.dot(lhs, rhs, preferred_element_type=F32).astype(BF16))
    mt_a[...] = jnp.concatenate(msegs, axis=0).T

    zero_tile = jnp.zeros((D // 2, 128), I32)
    kp_s[0, 0:D // 2, :] = zero_tile
    vp_s[0, 0:D // 2, :] = zero_tile
    lane3 = lax.broadcasted_iota(I32, (1, 8, 128), 2)
    lane2 = lax.broadcasted_iota(I32, (8, 128), 1)
    scale = (DH ** -0.5) * LOG2E

    def shifted(ext, w):
        if w == 0:
            return ext[1:]
        r = pltpu.roll(ext, DIL * w, 2)
        return jnp.where(lane3 < DIL * w, r[:-1], r[1:])

    def out_copy(i):
        return pltpu.make_async_copy(outbuf.at[i], out_hbm.at[pl.ds(i * SB, SB), :], sem_out.at[i])

    def qrows(r0, tiles=slice(None)):
        return pltpu.bitcast(q_s[tiles, pl.ds(r0, 8, stride=DH), :], F32)

    def block(i, last):
        t0 = i * T
        prev = (i + NB - 1) % NB

        for c in range(9):
            wds = jnp.concatenate([q_s[j, 64 * c:64 * c + 64, :] for j in range(T)], axis=1)
            outbuf[prev, :, 128 * c:128 * c + 128] = pltpu.bitcast(wds, BF16).T

        for r in range(0, D, D // 2):
            qa = _phi(jnp.dot(wt_a[r:r + D // 2, :], xa[i], preferred_element_type=F32))
            for j in range(T):
                q_s[j, r:r + D // 2, :] = pltpu.bitcast(qa[:, 128 * j:128 * j + 128], I32)
        for g in range(4):
            den = None
            for dh in range(DH):
                r0 = GR * g + 8 * dh
                pr = qrows(GR * g + dh) * zp[r0:r0 + 8, :][None]
                den = pr if den is None else den + pr
            inv = 1.0 / (den + 1e-6)
            for m in range(DH // 2):
                lo = qrows(GR * g + 2 * m) * inv
                hi = qrows(GR * g + 2 * m + 1) * inv
                a_s[:, pl.ds(GR * g + 2 * m, 8, stride=DH), :] = lo
                a_s[:, pl.ds(GR * g + 2 * m + 1, 8, stride=DH), :] = hi

        x = xb[i]
        for g in range(4):
            r, rw, rq = GR * g, GR // 2 * g, QSTEP * g
            q, k, v = [jnp.dot(wt_b[c * D + r:c * D + r + GR, :], x, preferred_element_type=F32) for c in range(3)]
            kvp = pltpu.bitcast(jnp.concatenate([k, v], axis=0).astype(BF16), I32)
            for j in range(T):
                lanes = slice(128 * j, 128 * j + 128)
                q_s[j, rq:rq + GR, :] = pltpu.bitcast(q[:, lanes], I32)
                kp_s[t0 + 1 + j, rw:rw + GR // 2, :] = kvp[0:GR // 2, lanes]
                vp_s[t0 + 1 + j, rw:rw + GR // 2, :] = kvp[GR // 2:GR, lanes]

            if last and g == 3:
                out_copy(prev).start()
                out_copy(0).wait()

            for sb in range(T // TS):
                tl = pl.ds(sb * TS, TS)
                te = pl.ds(t0 + sb * TS, TS + 1)
                acc = [None] * W
                for m in range(DH // 2):
                    ext = kp_s[te, pl.ds(rw + m, 8, stride=DH // 2), :]
                    qlo = qrows(rq + 2 * m, tl)
                    qhi = qrows(rq + 2 * m + 1, tl)
                    for w in range(W):
                        klo, khi = _unpack(shifted(ext, w))
                        pr = qlo * klo + qhi * khi
                        acc[w] = pr if acc[w] is None else acc[w] + pr
                ls = []
                for w in range(W):
                    l = acc[w] * scale
                    if w > 0 and sb == 0:
                        l0 = jnp.where(lane2 + i * SB < DIL * w, -1e9 * LOG2E, l[0])
                        l = jnp.concatenate([l0[None], l[1:]], axis=0)
                    ls.append(l)
                mx = ls[0]
                for w in range(1, W):
                    mx = jnp.maximum(mx, ls[w])
                es = [jnp.exp2(l - mx) for l in ls]
                ssum = es[0]
                for w in range(1, W):
                    ssum = ssum + es[w]
                inv = 1.0 / ssum
                ps = [e * inv for e in es]
                for m in range(DH // 2):
                    ext = vp_s[te, pl.ds(rw + m, 8, stride=DH // 2), :]
                    olo = ohi = None
                    for w in range(W):
                        vlo, vhi = _unpack(shifted(ext, w))
                        olo = ps[w] * vlo if olo is None else olo + ps[w] * vlo
                        ohi = ps[w] * vhi if ohi is None else ohi + ps[w] * vhi
                    o_s[tl, pl.ds(r + 2 * m, 8, stride=DH), :] = olo
                    o_s[tl, pl.ds(r + 2 * m + 1, 8, stride=DH), :] = ohi

        a_in = jnp.concatenate([a_s[j, 0:D, :].astype(BF16) for j in range(T)], axis=1)
        b_in = jnp.concatenate([o_s[j, 0:D, :].astype(BF16) for j in range(T)], axis=1)
        oa = jnp.dot(mt_a[...], a_in, preferred_element_type=F32).astype(BF16)

        def b_out(r0, r1):
            return jnp.dot(wot_b[r0:r1, :], b_in, preferred_element_type=F32).astype(BF16)

        if not last:
            ot = pltpu.bitcast(jnp.concatenate([oa, b_out(0, D)], axis=0), I32)
            for j in range(T):
                q_s[j, 0:D, :] = ot[:, 128 * j:128 * j + 128]

            @pl.when(i > 0)
            def _():
                out_copy(prev).start()
            return

        cps = [pltpu.make_async_copy(outbuf.at[i, :, pl.ds(c0, nc)],
                                     out_hbm.at[pl.ds(i * SB, SB), pl.ds(c0, nc)], sem_out.at[NB - 1 + k])
               for k, (c0, nc) in enumerate([(0, 512), (512, 256), (768, 256), (1024, 128)])]
        ob0 = b_out(0, 192)
        outbuf[i, :, 0:512] = oa[0:512, :].T
        cps[0].start()
        out_copy(1).wait()
        ob1 = b_out(192, 448)
        outbuf[i, :, 512:768] = jnp.concatenate([oa[512:D, :], ob0], axis=0).T
        cps[1].start()
        out_copy(2).wait()
        ob2 = b_out(448, D)
        outbuf[i, :, 768:1024] = ob1.T
        cps[2].start()
        cps[0].wait()
        outbuf[i, :, 1024:1152] = ob2.T
        cps[3].start()
        for c in cps[1:]:
            c.wait()

    q_s[:, 0:D, :] = jnp.zeros((T, D, 128), I32)

    def loop_body(i, carry):
        block(i, False)
        return carry

    lax.fori_loop(0, NB - 1, loop_body, 0)
    block(NB - 1, True)


@jax.jit
def pallas_concat_heads__linear_attn_block__sliding_local_dilated__prompt_kernel(
    A_x: jax.Array,
    A_wqkv: jax.Array,
    A_wo: jax.Array,
    B_x: jax.Array,
    B_wqkv: jax.Array,
    B_wo: jax.Array,
):
    xa_t = jnp.swapaxes(A_x, 1, 2).reshape(D, S)
    xb_t = jnp.swapaxes(B_x, 1, 2).reshape(D, S)
    any_spec = pl.BlockSpec(memory_space=pl.ANY)
    vm = pltpu.VMEM
    scratch = [
        vm((NB, D, SB), BF16), vm((NB, D, SB), BF16),
        vm((D, 3 * D), BF16), vm((D, 3 * D), BF16), vm((D, D), BF16), vm((D, D), BF16),
        vm((2 * D, D), BF16), vm((3 * D, D), BF16), vm((D, D), BF16), vm((D, D), BF16),
        vm((D, 512), F32), vm((D - 512, D), F32), vm((D, 128), F32),
        vm((DP, 128), F32), vm((D, 128), F32),
        vm((T, DP, 128), I32),
        vm((1 + S // 128, DP // 2, 128), I32), vm((1 + S // 128, DP // 2, 128), I32),
        vm((T, DP, 128), F32), vm((T, DP, 128), F32),
        vm((NB, SB, 2 * D), BF16),
        pltpu.SemaphoreType.DMA((11 + 2 * NB,)), pltpu.SemaphoreType.DMA((NB + 3,)),
    ]
    out = pl.pallas_call(
        _kernel,
        out_shape=jax.ShapeDtypeStruct((S, 2 * D), BF16),
        in_specs=[any_spec] * 6,
        out_specs=any_spec,
        scratch_shapes=scratch,
        compiler_params=pltpu.CompilerParams(
            vmem_limit_bytes=100 * 1024 * 1024, disable_semaphore_checks=True),
    )(xa_t, A_wqkv, A_wo, xb_t, B_wqkv, B_wo)
    return out.reshape(1, S, 2 * D)
```
